```python
import os as _os
_os.environ.setdefault("JAX_PLATFORMS", "cpu")
import jax
import jax.numpy as jnp

def _softmax(x, axis=-1):
    return jax.nn.softmax(x, axis=axis)
def _gelu(x):
    return jax.nn.gelu(x, approximate=True)
def _silu(x):
    return jax.nn.silu(x)
def _sigmoid(x):
    return jax.nn.sigmoid(x)
def _layernorm(x, axis=-1, eps=1e-5):
    m = jnp.mean(x, axis=axis, keepdims=True)
    v = jnp.var(x, axis=axis, keepdims=True)
    return (x - m) / jnp.sqrt(v + eps)
def _scatter_add(tgt, idx, src, axis=0):
    return tgt.at[idx].add(src)
def _segment_sum(src, seg, n):
    return jax.ops.segment_sum(src, seg, n)
class _Rng:
    def __init__(self, key):
        self._k = key
    def _next(self):
        self._k, sub = jax.random.split(self._k)
        return sub
    def normal(self, shape):
        return jax.random.normal(self._next(), shape, dtype=jnp.bfloat16)
    def randint(self, lo, hi, shape):
        return jax.random.randint(self._next(), shape, lo, hi, dtype=jnp.int32)
    def uniform(self, shape, lo=0.0, hi=1.0):
        return jax.random.uniform(self._next(), shape, jnp.bfloat16, lo, hi)
    def permutation(self, n):
        return jax.random.permutation(self._next(), n)


kernel_name = 'standalone__se_block__vision'

def setup_inputs():
    _rng = _Rng(jax.random.key(int.from_bytes(__import__("os").urandom(4), "little")))
    _w = (lambda a: (lambda t: t.astype(jnp.bfloat16) if jnp.issubdtype(t.dtype, jnp.floating) else t)(jnp.asarray(a)))
    H = W = 384
    C = 192; r = max(C // 16, 4)
    return {
        "x": _w((lambda *s: _rng.normal(s) * 0.8)(1, H, W, C)),
        "w_down": _w((lambda *s: _rng.normal(s) * 0.8)(C, r)),
        "w_up": _w((lambda *s: _rng.normal(s) * 0.8)(r, C)),
    }

def reference(x, w_down, w_up):
    s = x.mean(axis=(1, 2))
    s = _sigmoid(_silu(s @ w_down) @ w_up)
    return x * s[:, None, None, :]
```

```python
import functools

import jax
import jax.numpy as jnp
import jax.experimental.pallas as pl
import jax.experimental.pallas.tpu as pltpu
from jax import lax

_LANES = 128
_STREAMS = 6
_BULK = (256, 88, 24)
_HEAD = (10, 4, 2)
_TAIL = (13, 3)
_NUM_SEMS = 3


def _tree_sum(vs):
    vs = list(vs)
    while len(vs) > 1:
        vs = [vs[i] + vs[i + 1] if i + 1 < len(vs) else vs[i] for i in range(0, len(vs), 2)]
    return vs[0]


def _se_kernel(x_hbm, wd_hbm, wu_hbm, o_hbm, buf, wd_v, wu_v, wd_cols, wu_cols, scale, sems):
    f32 = jnp.float32
    H, slab, _ = x_hbm.shape
    R, C = wd_hbm.shape
    G = C // 8
    K = slab // C
    piece = 2 * K * 8
    inv_n = 1.0 / (H * K * _LANES)

    n_tail = sum(_TAIL)
    spans = []
    for sizes, h0, r0, r1 in (
        (_BULK, 0, 0, slab),
        (_HEAD, H - n_tail, 0, slab - piece),
        (_TAIL, H - n_tail, slab - piece, slab),
    ):
        for n in sizes:
            spans.append((h0, n, r0, r1))
            h0 += n
    reads = []
    for i, (h0, n, r0, r1) in enumerate(spans):
        idx = (pl.ds(h0, n), pl.ds(r0, r1 - r0))
        reads.append(pltpu.make_async_copy(x_hbm.at[idx], buf.at[idx], sems.at[i % _NUM_SEMS]))
    wd_copy = pltpu.make_async_copy(wd_hbm, wd_v, sems.at[_NUM_SEMS - 1])
    wu_copy = pltpu.make_async_copy(wu_hbm, wu_v, sems.at[_NUM_SEMS - 1])
    wd_copy.start()
    wu_copy.start()
    for i in range(_NUM_SEMS - 1):
        reads[i].start()
    wd_copy.wait()
    wu_copy.wait()
    reads[_NUM_SEMS - 1].start()

    def wait_read(i):
        reads[i].wait()
        if i + _NUM_SEMS < len(reads):
            reads[i + _NUM_SEMS].start()

    wd = wd_v[...]
    wd_mean = wd.astype(f32) * inv_n
    for j in range(16):
        c = C - 16 + j
        wd_cols[j] = jnp.broadcast_to(wd_mean[:, c : c + 1], (R, _LANES))
    wu_t = wu_v[...].astype(f32).T
    for r in range(R):
        wu_cols[r] = jnp.broadcast_to(wu_t[:, r : r + 1], (C, _LANES))

    def add_rows(r0, r1, h, accs):
        accs = list(accs)
        for i in range(r0 // 16, r1 // 16):
            v = buf[h, pl.ds(16 * i, 16), :].astype(f32)
            g0, g1 = (2 * i) // K, (2 * i + 1) // K
            accs[g0] = accs[g0] + v[0:8]
            accs[g1] = accs[g1] + v[8:16]
        return tuple(accs)

    accs = tuple(jnp.zeros((8, _LANES), f32) for _ in range(G))
    n_pre = len(_BULK) + len(_HEAD)
    for i in range(n_pre):
        wait_read(i)
        h0, n, r0, r1 = spans[i]
        unroll = 4 if n % 4 == 0 and n > 4 else 1
        accs = lax.fori_loop(h0, h0 + n, functools.partial(add_rows, r0, r1), accs, unroll=unroll)

    total = jnp.concatenate(accs, axis=0)
    hi = total.astype(jnp.bfloat16)
    lo = (total - hi.astype(f32)).astype(jnp.bfloat16)
    hidden = jnp.dot(wd, hi, preferred_element_type=f32) + jnp.dot(wd, lo, preferred_element_type=f32)
    hidden = hidden * inv_n

    tail = ([], [])
    for i in range(n_pre, len(reads)):
        h0, n, r0, r1 = spans[i]
        if i == len(reads) - 1:
            cols = [wd_cols[j] for j in range(16)]
        wait_read(i)
        new = ([], [])
        for h in range(h0, h0 + n):
            for j in range(K):
                v = buf[h, pl.ds(r0 + 16 * j, 16), :].astype(f32)
                new[(2 * j) // K].append(v[0:8])
                new[(2 * j + 1) // K].append(v[8:16])
        tail = tuple([_tree_sum(new[g] + tail[g])] for g in range(2))

    terms = [
        jnp.broadcast_to(tail[g][0][j : j + 1], (R, _LANES)) * cols[8 * g + j]
        for g in range(2)
        for j in range(8)
    ]
    hidden = jnp.sum(_tree_sum([hidden] + terms), axis=1, keepdims=True)

    hidden = jnp.broadcast_to(hidden, (R, _LANES))
    act = hidden * jax.nn.sigmoid(hidden)
    acts = [jnp.broadcast_to(act[r : r + 1], (16, _LANES)) for r in range(R)]

    streams = buf.reshape(o_hbm.shape)

    def scale_and_write(h, q, s):
        s0, s1 = s[0:8], s[8:16]
        for i in range(K):
            si = jnp.concatenate([s0 if 2 * i < K else s1, s0 if 2 * i + 1 < K else s1], axis=0)
            rows = pl.ds(q * piece + 16 * i, 16)
            for a in range(_STREAMS):
                streams[a, h, rows, :] = (streams[a, h, rows, :].astype(f32) * si).astype(buf.dtype)
        idx = (slice(None), h, pl.ds(q * piece, piece))
        pltpu.make_async_copy(streams.at[idx], o_hbm.at[idx], sems.at[0]).start()

    for q in range(G // 2):
        cols = [wu_cols[r, pl.ds(16 * q, 16), :] for r in range(R)]
        s = jax.nn.sigmoid(_tree_sum([acts[r] * cols[r] for r in range(R)]))
        scale[pl.ds(16 * q, 16), :] = s
        scale_and_write(0, q, s)

    def write_row(h, carry):
        for q in range(G // 2):
            scale_and_write(h, q, scale[pl.ds(16 * q, 16), :])
        return carry

    lax.fori_loop(1, H // _STREAMS, write_row, 0)
    pltpu.make_async_copy(buf, buf, sems.at[0]).wait()


@jax.jit
def pallas_standalone__se_block__vision_kernel(
    x: jax.Array,
    w_down: jax.Array,
    w_up: jax.Array,
):
    B, H, W, C = x.shape
    R = w_down.shape[1]
    G, K = C // 8, W // _LANES
    slab = C * K
    assert B == 1 and C % 16 == 0 and W % _LANES == 0 and H % _STREAMS == 0
    assert sum(_BULK) + sum(_TAIL) == H and sum(_HEAD) == sum(_TAIL)

    tiles = x.transpose(0, 1, 3, 2).reshape(H, G, 8, K, _LANES).transpose(0, 1, 3, 2, 4)

    out = pl.pallas_call(
        _se_kernel,
        out_shape=jax.ShapeDtypeStruct((_STREAMS, H // _STREAMS, slab, _LANES), x.dtype),
        in_specs=[pl.BlockSpec(memory_space=pltpu.HBM)] * 3,
        out_specs=pl.BlockSpec(memory_space=pltpu.HBM),
        scratch_shapes=[
            pltpu.VMEM((H, slab, _LANES), x.dtype),
            pltpu.VMEM((R, C), w_down.dtype),
            pltpu.VMEM((R, C), w_up.dtype),
            pltpu.VMEM((16, R, _LANES), jnp.float32),
            pltpu.VMEM((R, C, _LANES), jnp.float32),
            pltpu.VMEM((C, _LANES), jnp.float32),
            pltpu.SemaphoreType.DMA((_NUM_SEMS,)),
        ],
        compiler_params=pltpu.CompilerParams(vmem_limit_bytes=100 * 1024 * 1024),
    )(tiles.reshape(H, slab, _LANES), w_down.T, w_up)

    out = out.reshape(H, G, K, 8, _LANES).transpose(0, 1, 3, 2, 4).reshape(B, H, C, W)
    return out.transpose(0, 1, 3, 2)
```

```python
import functools

import jax
import jax.numpy as jnp
import jax.experimental.pallas as pl
import jax.experimental.pallas.tpu as pltpu
from jax import lax

_LANES = 128
_BULK = (256, 88, 24)
_HEAD = (10, 4, 2)
_TAIL = (13, 3)
_NUM_SEMS = 3
_STREAMS = 6
_STREAM_ROWS = 4096
_PIECE_ROWS = 64


def _tree_sum(vs):
    vs = list(vs)
    while len(vs) > 1:
        vs = [vs[i] + vs[i + 1] if i + 1 < len(vs) else vs[i] for i in range(0, len(vs), 2)]
    return vs[0]


def _se_kernel(x_hbm, wd_hbm, wu_hbm, o_hbm, buf, wd_v, wu_v, wd_cols, wu_cols, table, sems):
    f32 = jnp.float32
    H, slab, _ = x_hbm.shape
    R, C = wd_hbm.shape
    G = C // 8
    K = slab // C
    tail_rows = 2 * K * 8
    inv_n = 1.0 / (H * K * _LANES)

    n_tail = sum(_TAIL)
    spans = []
    for sizes, h0, r0, r1 in (
        (_BULK, 0, 0, slab),
        (_HEAD, H - n_tail, 0, slab - tail_rows),
        (_TAIL, H - n_tail, slab - tail_rows, slab),
    ):
        for n in sizes:
            spans.append((h0, n, r0, r1))
            h0 += n
    reads = []
    for i, (h0, n, r0, r1) in enumerate(spans):
        idx = (pl.ds(h0, n), pl.ds(r0, r1 - r0))
        reads.append(pltpu.make_async_copy(x_hbm.at[idx], buf.at[idx], sems.at[i % _NUM_SEMS]))
    wd_copy = pltpu.make_async_copy(wd_hbm, wd_v, sems.at[_NUM_SEMS - 1])
    wu_copy = pltpu.make_async_copy(wu_hbm, wu_v, sems.at[_NUM_SEMS - 1])
    wd_copy.start()
    wu_copy.start()
    for i in range(_NUM_SEMS - 1):
        reads[i].start()
    wd_copy.wait()
    wu_copy.wait()
    reads[_NUM_SEMS - 1].start()

    def wait_read(i):
        reads[i].wait()
        if i + _NUM_SEMS < len(reads):
            reads[i + _NUM_SEMS].start()

    wd = wd_v[...]
    wd_mean = wd.astype(f32) * inv_n
    for j in range(16):
        c = C - 16 + j
        wd_cols[j] = jnp.broadcast_to(wd_mean[:, c : c + 1], (R, _LANES))
    wu_t = wu_v[...].astype(f32).T
    for r in range(R):
        wu_cols[r] = jnp.broadcast_to(wu_t[:, r : r + 1], (C, _LANES))

    def add_rows(r0, r1, h, accs):
        accs = list(accs)
        for i in range(r0 // 16, r1 // 16):
            v = buf[h, pl.ds(16 * i, 16), :].astype(f32)
            g0, g1 = (2 * i) // K, (2 * i + 1) // K
            accs[g0] = accs[g0] + v[0:8]
            accs[g1] = accs[g1] + v[8:16]
        return tuple(accs)

    accs = tuple(jnp.zeros((8, _LANES), f32) for _ in range(G))
    n_pre = len(_BULK) + len(_HEAD)
    for i in range(n_pre):
        wait_read(i)
        h0, n, r0, r1 = spans[i]
        if n <= 2:
            for h in range(h0, h0 + n):
                accs = add_rows(r0, r1, h, accs)
        else:
            unroll = 4 if n % 4 == 0 and n > 4 else 1
            accs = lax.fori_loop(h0, h0 + n, functools.partial(add_rows, r0, r1), accs, unroll=unroll)

    total = jnp.concatenate(accs, axis=0)
    hi = total.astype(jnp.bfloat16)
    lo = (total - hi.astype(f32)).astype(jnp.bfloat16)
    hidden = jnp.dot(wd, hi, preferred_element_type=f32) + jnp.dot(wd, lo, preferred_element_type=f32)
    hidden = hidden * inv_n

    tail = ([], [])
    for i in range(n_pre, len(reads)):
        h0, n, r0, r1 = spans[i]
        if i == len(reads) - 1:
            cols = [wd_cols[j] for j in range(16)]
        wait_read(i)
        new = ([], [])
        for h in range(h0, h0 + n):
            for j in range(K):
                v = buf[h, pl.ds(r0 + 16 * j, 16), :].astype(f32)
                new[(2 * j) // K].append(v[0:8])
                new[(2 * j + 1) // K].append(v[8:16])
        tail = tuple([_tree_sum(new[g] + tail[g])] for g in range(2))

    terms = [
        jnp.broadcast_to(tail[g][0][j : j + 1], (R, _LANES)) * cols[8 * g + j]
        for g in range(2)
        for j in range(8)
    ]
    hidden = jnp.sum(_tree_sum([hidden] + terms), axis=1, keepdims=True)

    hidden = jnp.broadcast_to(hidden, (R, _LANES))
    act = hidden * jax.nn.sigmoid(hidden)
    acts = [jnp.broadcast_to(act[r : r + 1], (8, _LANES)) for r in range(R)]

    scales = {}

    def group_scale(g):
        if g not in scales:
            z = _tree_sum([acts[r] * wu_cols[r, pl.ds(8 * g, 8), :] for r in range(R)])
            scales[g] = jax.nn.sigmoid(z)
            for row in range(8 * K * g, table.shape[0], slab):
                for k in range(K):
                    if row + 8 * k < table.shape[0]:
                        table[pl.ds(row + 8 * k, 8), :] = scales[g]
        return scales[g]

    streams = buf.reshape(o_hbm.shape)
    kinds = slab // _PIECE_ROWS
    pieces = _STREAM_ROWS // _PIECE_ROWS

    first_steps = kinds - _STREAMS + 1
    for j in range(first_steps):
        width = 1 if j == 0 else _STREAMS
        for s0 in range(0, _STREAMS, width):
            for s in range(s0, s0 + width):
                for i in range(_PIECE_ROWS // 16):
                    tile = (s + j) % kinds * (_PIECE_ROWS // 8) + 2 * i
                    scale = jnp.concatenate([group_scale(tile // K), group_scale((tile + 1) // K)], axis=0)
                    rows = pl.ds(j * _PIECE_ROWS + 16 * i, 16)
                    streams[s, rows, :] = (streams[s, rows, :].astype(f32) * scale).astype(buf.dtype)
            idx = (pl.ds(s0, width), pl.ds(j * _PIECE_ROWS, _PIECE_ROWS))
            pltpu.make_async_copy(streams.at[idx], o_hbm.at[idx], sems.at[0]).start()

    def write_step(n, carry):
        s0 = n // pieces * _STREAMS
        j = n % pieces
        idx = (pl.ds(s0, _STREAMS), pl.ds(pl.multiple_of(j * _PIECE_ROWS, _PIECE_ROWS), _PIECE_ROWS))
        data = streams.at[idx]
        first = pl.multiple_of((s0 + j) % kinds * _PIECE_ROWS, _PIECE_ROWS)
        scale = table.at[pl.ds(first, _STREAMS * _PIECE_ROWS)]
        for s in range(_STREAMS):
            for i in range(_PIECE_ROWS // 16):
                rows = pl.ds(16 * i, 16)
                v = data[s, rows, :].astype(f32) * scale[pl.ds(s * _PIECE_ROWS + 16 * i, 16), :]
                data[s, rows, :] = v.astype(buf.dtype)
        pltpu.make_async_copy(data, o_hbm.at[idx], sems.at[0]).start()
        return carry

    lax.fori_loop(first_steps, o_hbm.shape[0] // _STREAMS * pieces, write_step, 0)
    pltpu.make_async_copy(buf, buf, sems.at[0]).wait()


@jax.jit
def pallas_standalone__se_block__vision_kernel(
    x: jax.Array,
    w_down: jax.Array,
    w_up: jax.Array,
):
    B, H, W, C = x.shape
    R = w_down.shape[1]
    G, K = C // 8, W // _LANES
    slab = C * K
    kinds = slab // _PIECE_ROWS
    assert B == 1 and C % 16 == 0 and W % _LANES == 0
    assert sum(_BULK) + sum(_TAIL) == H and sum(_HEAD) == sum(_TAIL)
    assert H * slab % (_STREAMS * _STREAM_ROWS) == 0 and slab % _PIECE_ROWS == 0
    assert _STREAM_ROWS // _PIECE_ROWS % kinds == 1 and kinds >= _STREAMS

    tiles = x.transpose(0, 1, 3, 2).reshape(H, G, 8, K, _LANES).transpose(0, 1, 3, 2, 4)

    out = pl.pallas_call(
        _se_kernel,
        out_shape=jax.ShapeDtypeStruct((H * slab // _STREAM_ROWS, _STREAM_ROWS, _LANES), x.dtype),
        in_specs=[pl.BlockSpec(memory_space=pltpu.HBM)] * 3,
        out_specs=pl.BlockSpec(memory_space=pltpu.HBM),
        scratch_shapes=[
            pltpu.VMEM((H, slab, _LANES), x.dtype),
            pltpu.VMEM((R, C), w_down.dtype),
            pltpu.VMEM((R, C), w_up.dtype),
            pltpu.VMEM((16, R, _LANES), jnp.float32),
            pltpu.VMEM((R, C, _LANES), jnp.float32),
            pltpu.VMEM(((kinds + _STREAMS - 1) * _PIECE_ROWS, _LANES), jnp.float32),
            pltpu.SemaphoreType.DMA((_NUM_SEMS,)),
        ],
        compiler_params=pltpu.CompilerParams(vmem_limit_bytes=100 * 1024 * 1024),
    )(tiles.reshape(H, slab, _LANES), w_down.T, w_up)

    out = out.reshape(H, G, K, 8, _LANES).transpose(0, 1, 3, 2, 4).reshape(B, H, C, W)
    return out.transpose(0, 1, 3, 2)
```

```python
import functools

import jax
import jax.numpy as jnp
import jax.experimental.pallas as pl
import jax.experimental.pallas.tpu as pltpu
from jax import lax

_LANES = 128
_BULK = (320, 52)
_HEAD = (8, 3, 1)
_TAIL = (10, 2)
_STREAMS = 6
_STREAM_ROWS = 4096
_PIECE_ROWS = 64


def _tree_sum(vs):
    vs = list(vs)
    while len(vs) > 1:
        vs = [vs[i] + vs[i + 1] if i + 1 < len(vs) else vs[i] for i in range(0, len(vs), 2)]
    return vs[0]


def _se_body(x_hbm, wd_hbm, wu_hbm, o_hbm, buf, wd_v, wu_v, wd_cols, wu_cols, table, read_sems, write_sem):
    f32 = jnp.float32
    H, slab, _ = x_hbm.shape
    R, C = wd_hbm.shape
    K = slab // C
    pair = 16 * K
    inv_n = 1.0 / (H * K * _LANES)

    h_tail = H - sum(_TAIL)
    spans = []
    for sizes, h0, r0, r1 in (
        (_BULK, 0, 0, slab),
        (_HEAD, h_tail, 0, slab - pair),
        (_TAIL, h_tail, slab - pair, slab),
    ):
        for n in sizes:
            spans.append((h0, n, r0, r1))
            h0 += n
    reads = []
    for i, (h0, n, r0, r1) in enumerate(spans):
        idx = (pl.ds(h0, n), pl.ds(r0, r1 - r0))
        reads.append(pltpu.make_async_copy(x_hbm.at[idx], buf.at[idx], read_sems.at[i]))
    wd_copy = pltpu.make_async_copy(wd_hbm, wd_v, read_sems.at[len(reads)])
    wu_copy = pltpu.make_async_copy(wu_hbm, wu_v, read_sems.at[len(reads) + 1])
    for copy in [wd_copy, wu_copy] + reads:
        copy.start()
    wd_copy.wait()
    wu_copy.wait()

    wd = wd_v[...]
    wd_mean = wd.astype(f32) * inv_n
    for j in range(16):
        c = C - 16 + j
        wd_cols[j] = jnp.broadcast_to(wd_mean[:, c : c + 1], (R, _LANES))
    wu_t = wu_v[...].astype(f32).T
    for r in range(R):
        wu_cols[r] = jnp.broadcast_to(wu_t[:, r : r + 1], (C, _LANES))

    def row_sum(h, q):
        tiles = []
        for i in range(K):
            v = buf[h, pl.ds(pair * q + 16 * i, 16), :].astype(f32)
            tiles += [v[0:8], v[8:16]]
        return jnp.concatenate([_tree_sum(tiles[:K]), _tree_sum(tiles[K:])], axis=0)

    def add_row(nq, h, sums):
        return tuple(s + row_sum(h, q) if q < nq else s for q, s in enumerate(sums))

    sums = tuple(jnp.zeros((16, _LANES), f32) for _ in range(C // 16))
    n_head = len(_BULK) + len(_HEAD)
    for copy, (h0, n, _, r1) in zip(reads[:n_head], spans[:n_head]):
        copy.wait()
        if n == 1:
            sums = add_row(r1 // pair, h0, sums)
        else:
            unroll = 4 if n % 4 == 0 else 1
            sums = lax.fori_loop(h0, h0 + n, functools.partial(add_row, r1 // pair), sums, unroll=unroll)

    hi = [s.astype(wd.dtype) for s in sums]
    lo = [(s - t.astype(f32)).astype(wd.dtype) for s, t in zip(sums, hi)]
    hidden = jnp.dot(wd, jnp.concatenate(hi, axis=0), preferred_element_type=f32)
    hidden += jnp.dot(wd, jnp.concatenate(lo, axis=0), preferred_element_type=f32)
    hidden *= inv_n

    tail = []
    for copy, (h0, n, _, _) in zip(reads[n_head:], spans[n_head:]):
        copy.wait()
        tail = [_tree_sum([row_sum(h, C // 16 - 1) for h in range(h0, h0 + n)] + tail)]
    terms = [jnp.broadcast_to(tail[0][j : j + 1], (R, _LANES)) * wd_cols[j] for j in range(16)]
    hidden = jnp.sum(_tree_sum([hidden] + terms), axis=1, keepdims=True)

    hidden = jnp.broadcast_to(hidden, (R, _LANES))
    act = hidden * jax.nn.sigmoid(hidden)
    acts = [jnp.broadcast_to(act[r : r + 1], (8, _LANES)) for r in range(R)]

    scales = {}

    def scale_of(g):
        if g not in scales:
            z = _tree_sum([acts[r] * wu_cols[r, pl.ds(8 * g, 8), :] for r in range(R)])
            scales[g] = jax.nn.sigmoid(z)
        return scales[g]

    streams = buf.reshape(o_hbm.shape)
    pieces = _STREAM_ROWS // _PIECE_ROWS
    kinds = slab // _PIECE_ROWS

    first_steps = kinds - _STREAMS + 1
    tabled = 0
    for j in range(first_steps):
        width = 1 if j == 0 else _STREAMS
        for s0 in range(0, _STREAMS, width):
            for s in range(s0, s0 + width):
                for i in range(_PIECE_ROWS // 16):
                    tile = (s + j) * (_PIECE_ROWS // 8) + 2 * i
                    scale = jnp.concatenate([scale_of(tile // K), scale_of((tile + 1) // K)], axis=0)
                    rows = pl.ds(j * _PIECE_ROWS + 16 * i, 16)
                    streams[s, rows, :] = (streams[s, rows, :].astype(f32) * scale).astype(buf.dtype)
            idx = (pl.ds(s0, width), pl.ds(j * _PIECE_ROWS, _PIECE_ROWS))
            pltpu.make_async_copy(streams.at[idx], o_hbm.at[idx], write_sem).start()
            for g in range(tabled, len(scales)):
                for row in range(8 * K * g, table.shape[0], slab):
                    for k in range(row, min(row + 8 * K, table.shape[0]), 8):
                        table[pl.ds(k, 8), :] = scales[g]
            tabled = len(scales)
    assert tabled == C // 8

    def write_step(n, carry):
        s0 = n // pieces * _STREAMS
        j = n % pieces
        idx = (pl.ds(s0, _STREAMS), pl.ds(pl.multiple_of(j * _PIECE_ROWS, _PIECE_ROWS), _PIECE_ROWS))
        data = streams.at[idx]
        first = pl.multiple_of((s0 + j) % kinds * _PIECE_ROWS, _PIECE_ROWS)
        scale = table.at[pl.ds(first, _STREAMS * _PIECE_ROWS)]
        for s in range(_STREAMS):
            for i in range(_PIECE_ROWS // 16):
                rows = pl.ds(16 * i, 16)
                v = data[s, rows, :].astype(f32) * scale[pl.ds(s * _PIECE_ROWS + 16 * i, 16), :]
                data[s, rows, :] = v.astype(buf.dtype)
        pltpu.make_async_copy(data, o_hbm.at[idx], write_sem).start()
        return carry

    lax.fori_loop(first_steps, o_hbm.shape[0] // _STREAMS * pieces, write_step, 0)
    pltpu.make_async_copy(buf, buf, write_sem).wait()


def _se_kernel(*refs):
    n_reads = len(_BULK) + len(_HEAD) + len(_TAIL) + 2
    pl.run_scoped(
        functools.partial(_se_body, *refs),
        pltpu.SemaphoreType.DMA((n_reads,)),
        pltpu.SemaphoreType.DMA(()),
    )


@jax.jit
def pallas_standalone__se_block__vision_kernel(
    x: jax.Array,
    w_down: jax.Array,
    w_up: jax.Array,
):
    B, H, W, C = x.shape
    R = w_down.shape[1]
    G, K = C // 8, W // _LANES
    slab = C * K
    kinds = slab // _PIECE_ROWS
    assert B == 1 and C % 16 == 0 and W % _LANES == 0
    assert sum(_BULK) + sum(_TAIL) == H and sum(_HEAD) == sum(_TAIL)
    assert H * slab % (_STREAMS * _STREAM_ROWS) == 0 and slab % _PIECE_ROWS == 0
    assert _STREAM_ROWS // _PIECE_ROWS % kinds == 1 and kinds >= _STREAMS

    tiles = x.transpose(0, 1, 3, 2).reshape(H, G, 8, K, _LANES).transpose(0, 1, 3, 2, 4)

    out = pl.pallas_call(
        _se_kernel,
        out_shape=jax.ShapeDtypeStruct((H * slab // _STREAM_ROWS, _STREAM_ROWS, _LANES), x.dtype),
        in_specs=[pl.BlockSpec(memory_space=pltpu.HBM)] * 3,
        out_specs=pl.BlockSpec(memory_space=pltpu.HBM),
        scratch_shapes=[
            pltpu.VMEM((H, slab, _LANES), x.dtype),
            pltpu.VMEM((R, C), w_down.dtype),
            pltpu.VMEM((R, C), w_up.dtype),
            pltpu.VMEM((16, R, _LANES), jnp.float32),
            pltpu.VMEM((R, C, _LANES), jnp.float32),
            pltpu.VMEM(((kinds + _STREAMS - 1) * _PIECE_ROWS, _LANES), jnp.float32),
        ],
        compiler_params=pltpu.CompilerParams(vmem_limit_bytes=100 * 1024 * 1024),
    )(tiles.reshape(H, slab, _LANES), w_down.T, w_up)

    out = out.reshape(H, G, K, 8, _LANES).transpose(0, 1, 3, 2, 4).reshape(B, H, C, W)
    return out.transpose(0, 1, 3, 2)
```
